```python
import os as _os
_os.environ.setdefault("JAX_PLATFORMS", "cpu")
import jax
import jax.numpy as jnp

def _softmax(x, axis=-1):
    return jax.nn.softmax(x, axis=axis)
def _gelu(x):
    return jax.nn.gelu(x, approximate=True)
def _silu(x):
    return jax.nn.silu(x)
def _sigmoid(x):
    return jax.nn.sigmoid(x)
def _layernorm(x, axis=-1, eps=1e-5):
    m = jnp.mean(x, axis=axis, keepdims=True)
    v = jnp.var(x, axis=axis, keepdims=True)
    return (x - m) / jnp.sqrt(v + eps)
def _scatter_add(tgt, idx, src, axis=0):
    return tgt.at[idx].add(src)
def _segment_sum(src, seg, n):
    return jax.ops.segment_sum(src, seg, n)
class _Rng:
    def __init__(self, key):
        self._k = key
    def _next(self):
        self._k, sub = jax.random.split(self._k)
        return sub
    def normal(self, shape):
        return jax.random.normal(self._next(), shape, dtype=jnp.bfloat16)
    def randint(self, lo, hi, shape):
        return jax.random.randint(self._next(), shape, lo, hi, dtype=jnp.int32)
    def uniform(self, shape, lo=0.0, hi=1.0):
        return jax.random.uniform(self._next(), shape, jnp.bfloat16, lo, hi)
    def permutation(self, n):
        return jax.random.permutation(self._next(), n)


kernel_name = 'interleave_layers__linear_kernel_hedgehog__sliding_block__prompt'

def setup_inputs():
    _rng = _Rng(jax.random.key(int.from_bytes(__import__("os").urandom(4), "little")))
    _w = (lambda a: (lambda t: t.astype(jnp.bfloat16) if jnp.issubdtype(t.dtype, jnp.floating) else t)(jnp.asarray(a)))
    def _A_setup():
        B, S, D, H = 1, 2048, 448, 16
        Dh = D // H
        return {
            "x": _w((lambda *s: _rng.normal(s) * 0.05)(B, S, D)),
            "wqkv": _w((lambda *s: _rng.normal(s) * 0.4)(D, 3 * D)),
            "w_phi": _w((lambda *s: _rng.normal(s) * 0.4)(H, Dh, Dh) * (Dh ** -0.5)),
            "wo": _w((lambda *s: _rng.normal(s) * 0.05)(D, D)),
        }
    _A_in = _A_setup()

    def _B_setup():
        B, S, D = 1, 2048, 448
        return {
            "x": _w((lambda *s: _rng.normal(s) * 0.05)(B, S, D)),
            "wqkv": _w((lambda *s: _rng.normal(s) * 0.1)(D, 3 * D)),
            "wo": _w((lambda *s: _rng.normal(s) * 0.1)(D, D)),
        }
    _B_in = _B_setup()

    return {
        "A_x": _A_in["x"],
        "A_wqkv": _A_in["wqkv"],
        "A_w_phi": _A_in["w_phi"],
        "A_wo": _A_in["wo"],
        "B_x": _B_in["x"],
        "B_wqkv": _B_in["wqkv"],
        "B_wo": _B_in["wo"],
    }

def reference(A_x, A_wqkv, A_w_phi, A_wo, B_x, B_wqkv, B_wo):
    def _A_ref(x, wqkv, w_phi, wo):
        B, S, D = x.shape
        H = 16; Dh = D // H
        qkv = (lambda x, *d: x.transpose(*d))((x @ wqkv).reshape(B, S, 3, H, Dh), 2, 0, 3, 1, 4)
        q, k, v = qkv[0], qkv[1], qkv[2]
        pq = jnp.einsum("bhsd,hdf->bhsf", q, w_phi)
        pk = jnp.einsum("bhsd,hdf->bhsf", k, w_phi)
        phi_q = jnp.concatenate([_softmax(pq, axis=-1), _softmax(-pq, axis=-1)], axis=-1)
        phi_k = jnp.concatenate([_softmax(pk, axis=-1), _softmax(-pk, axis=-1)], axis=-1)
        kv = jnp.einsum("bhsf,bhsd->bhfd", phi_k, v)
        z  = jnp.einsum("bhsf->bhf", phi_k)
        num = jnp.einsum("bhqf,bhfd->bhqd", phi_q, kv)
        den = jnp.einsum("bhqf,bhf->bhq", phi_q, z)[..., None] + 1e-6
        o = num / den
        return (lambda x, *d: x.transpose(*d))(o, 0, 2, 1, 3).reshape(B, S, D) @ wo

    def _B_ref(x, wqkv, wo):
        B, S, D = x.shape
        H = 16; Dh = D // H; W = 256
        qkv = (lambda x, *d: x.transpose(*d))((x @ wqkv).reshape(B, S, 3, H, Dh), 2, 0, 3, 1, 4)
        q, k, v = qkv[0], qkv[1], qkv[2]
        scores = jnp.einsum("bhqd,bhkd->bhqk", q, k) * (Dh ** -0.5)
        idx = jnp.arange(S)
        mask = (idx[:, None] - idx[None, :] >= 0) & (idx[:, None] - idx[None, :] < W)
        scores = jnp.where(mask[None, None], scores, -1e9)
        p = _softmax(scores, axis=-1)
        o = jnp.einsum("bhqk,bhkd->bhqd", p, v)
        return (lambda x, *d: x.transpose(*d))(o, 0, 2, 1, 3).reshape(B, S, D) @ wo

    x = A_x
    x = x + _A_ref(_layernorm(x, axis=-1), A_wqkv, A_w_phi, A_wo)
    x = x + _B_ref(_layernorm(x, axis=-1), B_wqkv, B_wo)
    x = x + _A_ref(_layernorm(x, axis=-1), A_wqkv, A_w_phi, A_wo)
    x = x + _B_ref(_layernorm(x, axis=-1), B_wqkv, B_wo)
    return x
```

```python
import jax
import jax.numpy as jnp
import numpy as np
from jax import lax
import jax.experimental.pallas as pl
import jax.experimental.pallas.tpu as pltpu

S, D, H, DH, WIN = 2048, 448, 16, 28, 256
T = 512
MAPS_IN_FLIGHT = 2
SLABS_IN_FLIGHT = 2
TILES = (0, 2, 1, 3)
SCHEDULE = (
    's0 s1 s2 fold x1 s3 al00 x2 wav av00:7 x3 s4 av00 wak ak00 al01 av01+fk00 ak01 x4 s5 '
    'kv00 waq al02 fk01 ak02 aq00 al03 fk02 ak03+av02 av03 kv01 kv02 fq00 fk03 kv03 x5 wao '
    'wbk nu00 aq01 ao00+fq01 bl00 nu01 aq02 wbq bk00 ao01+wbv fq02 bv00+bl01 bq00 bt00+nu02 '
    'bv01+wbo ao02 bl02 bk01 bo00+bq01 al10 aq03 bk02 bt01+fq03,av10 bo01+ak10,fk10 bq02+kv10 '
    'nu03+al11 bv02 bt02+ao03,bl03 ak11 fk11 bo02+bk03 av11 al12 kv11+bq03,bv03 '
    'bt03+av12,ak12 fk12 aq10 bo03+kv12 fq10 al13 aq11 fq11 ak13+aq12 fk13 av13 kv13 '
    'nu10+nu11,aq13 ao10 fq12 nu12+bl10 ao11 bl11 bq10 bk10 bv10 fq13 ao12 bv11 '
    'bt10+bk11,bq11,nu13 ao13 bl12 bo10+bq12 bt11+bk12,bv12 bl13 bk13 bq13 bo11 bt12+bv13 '
    'bt13+bo12 bo13 '
)
NC = S // T
TPC = T // 128
HT, HD = TPC // 2, D // 2
LOG2E = float(np.log2(np.e))
BF, F32, I32 = jnp.bfloat16, jnp.float32, jnp.int32
NT_DIMS = (((1,), (1,)), ((), ()))


def _dot(a, b):
    return jnp.dot(a, b, preferred_element_type=F32)


def _iota(shape, dim):
    return lax.broadcasted_iota(I32, shape, dim)


def _zip16(x):
    n, m = x.shape[0] // 16, x.shape[1]
    if n == 1:
        return pltpu.bitcast(pltpu.pack_elementwise([x[:8], x[8:]], packed_dtype=BF), I32)
    x = x.reshape(n, 16, m)
    w = pltpu.pack_elementwise([x[:, :8].reshape(8 * n, m), x[:, 8:].reshape(8 * n, m)], packed_dtype=BF)
    return pltpu.bitcast(w, I32)


def _unzip16(w):
    halves = [pltpu.unpack_elementwise(w, index=i, packed_dtype=BF, unpacked_dtype=F32) for i in range(2)]
    n, m = w.shape[0] // 8, w.shape[1]
    return jnp.concatenate([z.reshape(n, 8, m) for z in halves], axis=1).reshape(16 * n, m)


def _bf(x):
    return pltpu.bitcast(x, BF)


def _recip(x):
    r = pl.reciprocal(x, approx=True)
    return r * (2.0 - x * r)


def _pair_allreduce(vs, op):
    r = _tree(vs, op)
    r = op(r, pltpu.roll(r, 4, 0))
    return op(r, pltpu.roll(r, 2, 0))


def _feature_map(p, pace):
    vs = _vregs(p)
    hi, lo = pace(_pair_allreduce(vs, jnp.maximum), _pair_allreduce(vs, jnp.minimum))
    p = p.reshape(7, 8, 128)
    es = jnp.exp2(p - hi), jnp.exp2(lo - p)
    return jnp.concatenate([e * _recip(_pair_allreduce(_vregs(e.reshape(56, 128)), jnp.add)) for e in es],
                           axis=0).reshape(112, 128)


def _pack(x):
    return pltpu.bitcast(x.astype(BF), I32)


def _vregs(x):
    return [x[r:r + 8] for r in range(0, x.shape[0], 8)]


def _tree(vs, op):
    while len(vs) > 1:
        vs = [op(*vs[i:i + 2]) if i + 1 < len(vs) else vs[i] for i in range(0, len(vs), 2)]
    return vs[0]


def _total(vs, f):
    acc = None
    for i in range(0, len(vs), 4):
        part = _tree([f(v) for v in vs[i:i + 4]], jnp.add)
        acc = part if acc is None else acc + part
    return _all_rows(acc, jnp.add)


def _all_rows(r, op):
    for k in (4, 2, 1):
        r = op(r, pltpu.roll(r, k, 0))
    return r


def _left(a11, a12, a21, a22):
    return a21 + a22, a22, a11, a11 + a12, a11 + a22, a12 - a22, a21 - a11


def _right(b11, b12, b21, b22):
    return b11, b21 - b11, b12 - b22, b22, b11 + b22, b21 + b22, b11 + b12


def _combine(i, j, m):
    if i != j:
        return m[0] + m[1] if i else m[2] + m[3]
    return ((m[2] - m[0]) + m[4]) + m[6] if i else ((m[1] - m[3]) + m[4]) + m[5]


class _Pacer:
    def __init__(self, zero):
        self.history = []
        self.zero = jnp.full((8, 128), zero, I32)

    def after(self, y):
        if y is None:
            return lambda *xs: xs
        bits = pltpu.bitcast(y, I32) & self.zero
        return lambda *xs: [pltpu.bitcast(pltpu.bitcast(x, I32) | bits, x.dtype) for x in xs]

    def finished(self, words):
        self.history.append(_tree(words, jnp.bitwise_or))

    def behind(self, depth):
        return self.after(self.history[-depth] if depth <= len(self.history) else None)


def _rows(x):
    return lambda r, pace: jnp.concatenate(x[r // 8:r // 8 + 2], axis=0)


def _operand(tiles, pacer=None):
    cols = []
    for u in range(HT):
        parts = []
        for r in range(0, HD, 16):
            if pacer and r % (HD // 2) == 0:
                yield
            pace = pacer and pacer.behind(SLABS_IN_FLIGHT)
            parts.append([_zip16(f) for f in _right(
                *(tiles[i](j, pace) for j in (r, r + HD) for i in (u, u + HT)))])
            if pacer:
                pacer.finished(parts[-1])
        cols.append([jnp.concatenate(p, axis=0) for p in zip(*parts)])
    return [_bf(jnp.concatenate(c, axis=1)) for c in zip(*cols)]


def _normed_operand(xs, pacer):
    means, scales, tiles = [], [None] * TPC, []
    for u in TILES:
        yield
        mean = _total(xs[u], lambda v: v) * (1.0 / D)
        if means:
            mean, = pacer.after(var)(mean)
        var = _total(xs[u], lambda v: lax.square(v - mean)) * (1.0 / D)
        means.append(mean)
        scales[u] = lax.rsqrt(var + 1e-5)
    for u, x in enumerate(xs):
        scale, = pacer.after(scales[u + HT] if u < HT else None)(scales[u])
        tiles.append(lambda r, pace, x=x, scale=scale, shift=means[TILES.index(u)] * scale: jnp.concatenate(
            [v * s - shift for s in pace(scale) for v in x[r // 8:r // 8 + 2]], axis=0))
    return (yield from _operand(tiles, pacer))


def _project(w, xb):
    ms, blocks = [], {}
    for i in range(7):
        yield
        ms.append(_dot(w[i], xb[i]))
        for ij in {1: [(1, 0)], 3: [(0, 1)], 5: [(0, 0)], 6: [(1, 1)]}.get(i, []):
            blocks[ij] = _combine(*ij, ms)

    def get(u, r0, n):
        r, c = r0 % HD, 128 * (u % HT)
        return blocks[r0 // HD, u // HT][r:r + n, c:c + 128]
    return get


def _kernel(zero_ref, x_hbm, wa_hbm, wphi_hbm, woa_hbm, wb_hbm, wob_hbm, out_hbm,
            xin, wav_raw, wak_raw, waq_raw, wphi, woa_raw, wb_raw, wob_raw, obuf, s_bufs, x_sem, w_sem, o_sem):
    x_copies = [pltpu.make_async_copy(x_hbm.at[:, pl.ds(c * T, T)], xin.at[c], x_sem.at[c])
                for c in range(NC)]
    o_copies = {(t, r): pltpu.make_async_copy(
        obuf.at[t, pl.ds(r, HD), :], out_hbm.at[pl.ds(r, HD), pl.ds(t * 128, 128)], o_sem.at[2 * t + r // HD])
        for t in range(S // 128) for r in (0, HD)}
    w_copies = {name: pltpu.make_async_copy(src, dst, w_sem.at[i]) for i, (name, src, dst) in enumerate(
        [('av', wa_hbm.at[:, pl.ds(896, D)], wav_raw), ('ak', wa_hbm.at[:, pl.ds(384, 512)], wak_raw),
         ('aq', wa_hbm.at[:, pl.ds(0, 512)], waq_raw), ('phi', wphi_hbm, wphi), ('ao', woa_hbm, woa_raw),
         ('b', wb_hbm, wb_raw), ('bo', wob_hbm, wob_raw)])}

    zero = zero_ref[0]
    s_bufs, pacer = list(s_bufs), _Pacer(zero)
    xres, kv, heads, feats, xb = {}, {}, {}, {}, {}
    xn, qs, kn, vt = {}, {}, {}, {}
    wts, bds = {}, []

    def project(name, xb):
        return _project(wts[name], xb)

    def fold_matrices():
        r, c_ = _iota((D, D), 0), _iota((D, D), 1)
        perm = jnp.where(r == (c_ & 15) * DH + (c_ >> 4), 1.0, 0.0).astype(BF)
        r, c_ = _iota((112, DH), 0), _iota((112, DH), 1)
        sel = jnp.where((jnp.where(r >= 56, r - 56, r) >> 1) == c_, 1.0, 0.0).astype(BF)
        r, c_ = _iota((112, 112), 0), _iota((112, 112), 1)
        lo = (jnp.where(r >= 56, 2, 0) + (r & 1)) * DH
        same = (c_ >= lo) & (c_ < lo + DH)
        w_copies['phi'].wait()
        wp = _dot(perm, wphi[...])
        for g in range(4):
            bd = lax.dot_general(sel, wp[112 * g:112 * g + 112].astype(BF), NT_DIMS,
                                 preferred_element_type=F32)
            bds.append(jnp.where(same, bd, 0.0).astype(BF))

    def weight(name, ref, c0, fold=False, scale=None):
        a0 = c0 // 128 * 128
        cols = []
        for j in (0, HD):
            w = ref[j:j + HD, a0:min(a0 + 512, ref.shape[1])]
            if name[1] == 'o':
                cols.append(_unzip16(pltpu.bitcast(_bf(_zip16(w.astype(F32))).T, I32)))
            else:
                cols.append(w.T[c0 - a0:c0 - a0 + D])
        if fold:
            cols = [jnp.concatenate([_dot(bds[g], w[112 * g:112 * g + 112]) for g in range(4)], axis=0)
                    for w in cols]
        cols = [w.astype(F32) * scale if scale else w.astype(F32) for w in cols]
        wts[name] = [f.astype(BF) for f in _left(*(w[i:i + HD] for i in (0, HD) for w in cols))]

    ones8 = jnp.ones((8, 128), F32)
    low4 = _iota((8, 128), 0) < 4
    order = [(u, p) for early in (True, False) for u in range(TPC) for p in range(8)
             if ((u < HT) != (p < 4)) == early]

    def feature_maps(l, c, name):
        get, phi = feats[name, c], {}
        for i, (u, p) in enumerate(order):
            if i % 4 == 0:
                yield
            f = _zip16(_feature_map(get(u, 56 * p, 56), pacer.behind(MAPS_IN_FLIGHT)))
            pacer.finished(_vregs(f))
            phi[u, p] = _bf(f)
        feats[name, c] = phi

    def residual(c, get, last=False):
        for u, p in order[::2]:
            x = jnp.concatenate(xres[c][u][7 * p:7 * p + 14], axis=0) + get(u, 56 * p, 112)
            if last:
                obuf[c * TPC + u, 56 * p:56 * p + 112, :] = _bf(_zip16(x))
                if p % 4:
                    o_copies[c * TPC + u, 56 * p - 112].start()
            else:
                xres[c][u][7 * p:7 * p + 14] = _vregs(x)

    def a_norm(l, c):
        if l == 0:
            xres[c] = [_vregs(_unzip16(pltpu.bitcast(xin[c, :, 128 * u:128 * u + 128], I32)))
                       for u in range(TPC)]
        xn[c] = yield from _normed_operand(xres[c], pacer)

    def a_features(l, c, name):
        get = feats[name, c] = yield from project(name, xn[c])
        if name == 'av':
            feats[name, c] = {(u, p): jnp.concatenate([get(u, 56 * p, 56), ones8], axis=0).astype(BF)
                              for u, p in order}

    def a_summary(l, c):
        v, phi = feats['av', c], feats['ak', c]
        for p in range(8):
            if p % 4 == 0:
                yield
            parts = [lax.dot_general(v[u, p], phi[u, p], NT_DIMS, preferred_element_type=F32) for u in range(TPC)]
            kv[l, p] = _tree(parts + ([kv[l, p]] if c else []), jnp.add)
        if c == NC - 1:
            r, c_ = _iota((64, 112), 0), _iota((64, 112), 1)
            second = ((r >= DH) & (r < 56)) | (r >= 60)
            keep = jnp.where(second, 1, 0) == ((c_ >> 1) & 1)
            for p in range(8):
                kv[l, p] = jnp.where(keep, kv[l, p], 0.0).astype(BF)

    def spread(rec):
        swp = pltpu.roll(rec, 4, 0)
        ra, rb = jnp.where(low4, rec, swp), jnp.where(low4, swp, rec)
        return [ra, ra, ra, rec, rb, rb, rb]

    def a_attend(l, c):
        outs, phi = [[] for _ in range(TPC)], feats['aq', c]
        for p in range(8):
            if p % 4 == 0:
                yield
            for u in range(TPC):
                nd = _vregs(_dot(kv[l, p], phi[u, p]))
                outs[u] += [n * s for n, s in zip(nd, spread(_recip(nd[7] + 1e-6)))]
        heads['ao', c] = yield from _operand([_rows(x) for x in outs])

    def output(l, c, name):
        residual(c, (yield from project(name, heads[name, c])), last=(l, name) == (1, 'bo'))

    def b_norm(l, c):
        xb[c] = yield from _normed_operand(xres[c], pacer)

    def b_keys(l, c):
        zpad = jnp.zeros((8, 128), I32)
        k = yield from project('bk', xb[c])
        for u, p in order[::2]:
            kt = jnp.concatenate([_zip16(k(u, 56 * p, 112)), zpad], axis=0)
            kn[l, p // 2, c * TPC + u] = _pack(_unzip16(pltpu.bitcast(_bf(kt).T, I32)))

    def b_queries(l, c):
        q = yield from project('bq', xb[c])
        for u, p in order[::2]:
            qs[p // 2, c * TPC + u] = (_zip16(q(u, 56 * p, 112)))

    def b_values(l, c):
        v = yield from project('bv', xb[c])
        for u, p in order:
            vp = v(u, 56 * p, 56)
            vt[l, 2 * p, c * TPC + u] = jnp.concatenate(
                [vp[0:24], jnp.where(low4, vp[24:32], 1.0)], axis=0).astype(BF)
            vt[l, 2 * p + 1, c * TPC + u] = jnp.concatenate(
                [jnp.where(low4, 1.0, vp[24:32]), vp[32:56]], axis=0).astype(BF)

    def head_of(f):
        return (jnp.where(f >= DH, 1, 0) + jnp.where(f >= 2 * DH, 1, 0) + jnp.where(f >= 3 * DH, 1, 0))

    def halves(lo_mask, hi_mask):
        return jnp.where(lo_mask, 0xFFFF, 0) | jnp.where(hi_mask, -0x10000, 0)

    r, lane = _iota((128, 128), 0), _iota((128, 128), 1)
    key = (r & -16) + 2 * (r & 7) + ((r >> 3) & 1)
    older = key > lane
    from_diag = (~older) & ((r >> 5) == (lane >> 5))
    r, lane = _iota((64, 128), 0), _iota((64, 128), 1)
    older_bits = halves(2 * r > lane, 2 * r + 1 > lane)
    newer_bits = ~older_bits
    f_lo = 2 * (r & -8) + (r & 7)
    plain_bits = [halves(head_of(f_lo) == j, head_of(f_lo + 8) == j) for j in range(4)]
    latin_bits = [halves(head_of(f_lo) == ((lane >> 5) ^ j), head_of(f_lo + 8) == ((lane >> 5) ^ j))
                  for j in range(4)]
    odd_group, high_group = (lane & 32) != 0, (lane & 64) != 0
    lane = _iota((16, 128), 1)
    k_head = head_of((lane & -16) + ((lane & 15) >> 1) + 8 * (lane & 1))

    def scores(l, t, g):
        q = jnp.concatenate([qs[g, t], jnp.zeros((8, 128), I32)], axis=0)
        if t >= 2:
            old, mid, new = (kn[l, g, i] for i in (t - 2, t - 1, t))
            ss = []
            for j in range(4):
                grp = k_head ^ j
                mix = [jnp.where(grp <= b, old[16 * b:16 * b + 16], new[16 * b:16 * b + 16]) for b in range(3)]
                pair = [jnp.where((grp & 1) == 0, new[b:b + 16], new[b + 16:b + 32]) for b in (0, 32)]
                diag = jnp.where(grp < 2, pair[0], pair[1])
                ss.append(_dot(_bf(jnp.concatenate([diag] + mix + [old[48:], mid], axis=0)),
                               _bf(q & latin_bits[j])))
        else:
            keys = _bf(jnp.concatenate([kn[l, g, i] for i in range(t, -1, -1)], axis=0))
            ss = [_dot(keys, _bf(q & plain_bits[j])) for j in range(4)]
        out = []
        for s in ss:
            if t >= 2:
                tiles = [jnp.where(from_diag, jnp.concatenate([s[:32]] * 4, axis=0), s[32:160]), s[160:]]
            else:
                tiles = [jnp.where(older, -1e30, s[:128])] + ([s[128:]] if t else [])
            bufs, top = [s_bufs.pop(0) for _ in tiles], []
            for buf, z in zip(bufs, tiles):
                buf[0] = z
                for r in range(0, 128, 32):
                    top = [_tree([jnp.max(z[r:r + 32].reshape(4, 8, 128), axis=0)] + top, jnp.maximum)]
            out.append((bufs, jnp.concatenate([_all_rows(top[0], jnp.maximum)] * 16, axis=0)))
        return out

    def softmax(t, ss):
        ps = [[_zip16(jnp.exp2(buf[zero] - top)) for buf in bufs] for bufs, top in ss]
        s_bufs.extend(buf for bufs, _ in ss for buf in bufs)
        if t >= 2:
            for bit, mask in ((1, odd_group), (2, high_group)):
                ps = [[jnp.where(mask, y, x) for x, y in zip(ps[j], ps[j ^ bit])] for j in range(4)]
        return ps

    def attend(l, t, g, ps):
        terms = [(t, 0, None)] if t < 2 else [(t - 2, 0, older_bits), (t, 0, newer_bits)]
        os_ = [None] * 4
        for tk, i, bits in terms + ([(t - 1, 1, None)] if t else []):
            for j, p in enumerate(ps):
                o = _dot(vt[l, 4 * g + j, tk], _bf(p[i] if bits is None else p[i] & bits))
                os_[j] = o if os_[j] is None else os_[j] + o
        outs = []
        for oa, ob in ((os_[0], os_[1]), (os_[2], os_[3])):
            oa, ob = _vregs(oa), _vregs(ob)
            rec = pltpu.roll(_recip(jnp.where(low4, ob[0], oa[3])), 4, 0)
            outs += [n * s for n, s in zip(oa[:3] + [jnp.where(low4, oa[3], ob[0])] + ob[1:], spread(rec))]
        return outs

    def b_attend(l, c):
        units = [(l, c * TPC + u, g) for u in TILES for g in range(4)]
        outs = [[] for _ in range(TPC)]
        ss = scores(*units[0])
        for unit, following in zip(units, units[1:] + [None]):
            ahead = following and scores(*following)
            ps = softmax(unit[1], ss)
            yield
            outs[unit[1] % TPC] += attend(*unit, ps)
            ss = ahead
        heads['bo', c] = yield from _operand([_rows(x) for x in outs])

    batches = [[w_copies['phi']], x_copies[:1], [w_copies['av']], [w_copies['ak'], x_copies[1]],
               x_copies[2:] + [w_copies['aq']], [w_copies[k] for k in ('ao', 'b', 'bo')]]
    weights = dict(av=(wav_raw, 0), ak=(wak_raw, 64, True, LOG2E), aq=(waq_raw, 0, True, LOG2E),
                   ao=(woa_raw, 0), bk=(wb_raw, D), bq=(wb_raw, 0, False, LOG2E * DH ** -0.5),
                   bv=(wb_raw, 2 * D), bo=(wob_raw, 0))
    stages = dict(al=a_norm, kv=a_summary, nu=a_attend, bl=b_norm, bk=b_keys, bq=b_queries,
                  bv=b_values, bt=b_attend)

    def run(names):
        for name in names:
            if name[0] in 'sx':
                for cp in batches[int(name[1])]:
                    cp.start() if name[0] == 's' else cp.wait()
            elif name == 'fold':
                fold_matrices()
            elif name[0] == 'w':
                weight(name[1:], *weights[name[1:]])
            else:
                kind, l, c = name[:2], int(name[2]), int(name[3])
                if kind[0] == 'f':
                    yield from feature_maps(l, c, 'a' + kind[1])
                elif kind in stages:
                    yield from stages[kind](l, c) or ()
                else:
                    yield from (output if kind[1] == 'o' else a_features)(l, c, kind)

    paused = {}
    for group in SCHEDULE.split():
        if ':' in group or group in paused:
            name, _, n = group.partition(':')
            task = paused.setdefault(name, run([name]))
            for _ in range(int(n or 99)):
                next(task, None)
            continue
        main, _, fill = group.partition('+')
        fill = fill.split(',') if fill else []
        count, *steps = (dict(bt=16, kv=2, nu=2, al=8, bl=8, fk=8, fq=8).get(n[:2], 7 * (n[0] in 'ab'))
                         for n in [main] + fill)
        steps = sum(steps)
        filler = run(fill)
        next(filler, None)
        for i, _ in enumerate(run([main])):
            for _ in range(steps * (i + 1) // max(count, 1) - steps * i // max(count, 1)):
                next(filler, None)
        for _ in filler:
            pass

    for cp in o_copies.values():
        cp.wait()


@jax.jit
def pallas_interleave_layers__linear_kernel_hedgehog__sliding_block__prompt_kernel(
    A_x: jax.Array,
    A_wqkv: jax.Array,
    A_w_phi: jax.Array,
    A_wo: jax.Array,
    B_x: jax.Array,
    B_wqkv: jax.Array,
    B_wo: jax.Array,
):
    del B_x
    hbm = pl.BlockSpec(memory_space=pl.ANY)
    out = pl.pallas_call(
        _kernel,
        in_specs=[pl.BlockSpec(memory_space=pltpu.SMEM)] + [hbm] * 6,
        out_specs=hbm,
        out_shape=jax.ShapeDtypeStruct((D, S), BF),
        scratch_shapes=[
            pltpu.VMEM((NC, D, T), BF),
            pltpu.VMEM((D, D), BF),
            pltpu.VMEM((D, 512), BF),
            pltpu.VMEM((D, 512), BF),
            pltpu.VMEM((D, DH), BF),
            pltpu.VMEM((D, D), BF),
            pltpu.VMEM((D, 3 * D), BF),
            pltpu.VMEM((D, D), BF),
            pltpu.VMEM((S // 128, D, 128), BF),
            [pltpu.VMEM((1, 128, 128), F32)] * 64,
            pltpu.SemaphoreType.DMA((NC,)),
            pltpu.SemaphoreType.DMA((7,)),
            pltpu.SemaphoreType.DMA((S // 64,)),
        ],
        compiler_params=pltpu.CompilerParams(vmem_limit_bytes=100 * 1024 * 1024),
    )(
        np.zeros((1,), np.int32),
        A_x.reshape(S, D).T.astype(BF),
        A_wqkv.astype(BF),
        A_w_phi.transpose(1, 0, 2).reshape(D, DH).astype(BF),
        A_wo.astype(BF),
        B_wqkv.astype(BF),
        B_wo.astype(BF),
    )
    return out.T.reshape(1, S, D).astype(A_x.dtype)
```
